```python
import os as _os
_os.environ.setdefault("JAX_PLATFORMS", "cpu")
import jax
import jax.numpy as jnp

def _softmax(x, axis=-1):
    return jax.nn.softmax(x, axis=axis)
def _gelu(x):
    return jax.nn.gelu(x, approximate=True)
def _silu(x):
    return jax.nn.silu(x)
def _sigmoid(x):
    return jax.nn.sigmoid(x)
def _layernorm(x, axis=-1, eps=1e-5):
    m = jnp.mean(x, axis=axis, keepdims=True)
    v = jnp.var(x, axis=axis, keepdims=True)
    return (x - m) / jnp.sqrt(v + eps)
def _scatter_add(tgt, idx, src, axis=0):
    return tgt.at[idx].add(src)
def _segment_sum(src, seg, n):
    return jax.ops.segment_sum(src, seg, n)
class _Rng:
    def __init__(self, key):
        self._k = key
    def _next(self):
        self._k, sub = jax.random.split(self._k)
        return sub
    def normal(self, shape):
        return jax.random.normal(self._next(), shape, dtype=jnp.bfloat16)
    def randint(self, lo, hi, shape):
        return jax.random.randint(self._next(), shape, lo, hi, dtype=jnp.int32)
    def uniform(self, shape, lo=0.0, hi=1.0):
        return jax.random.uniform(self._next(), shape, jnp.bfloat16, lo, hi)
    def permutation(self, n):
        return jax.random.permutation(self._next(), n)


kernel_name = 'sequential_preLN__mha_block__dense_activation_mish__prompt'

def setup_inputs():
    _rng = _Rng(jax.random.key(int.from_bytes(__import__("os").urandom(4), "little")))
    _w = (lambda a: (lambda t: t.astype(jnp.bfloat16) if jnp.issubdtype(t.dtype, jnp.floating) else t)(jnp.asarray(a)))
    def _A_setup():
        B, S, D, H = 1, 2048, 576, 32
        return {
            "x": _w((lambda *s: _rng.normal(s) * 0.05)(B, S, D)),
            "wqkv": _w((lambda *s: _rng.normal(s) * 0.05)(D, 3 * D)),
            "wo": _w((lambda *s: _rng.normal(s) * 0.05)(D, D)),
        }
    _A_in = _A_setup()

    def _B_setup():
        B, S, D, F = 1, 2048, 576, 4608
        return {
            "x": _w((lambda *s: _rng.normal(s) * 0.05)(B, S, D)),
            "w1": _w((lambda *s: _rng.normal(s) * 1.6)(D, F) * (D ** -0.5)),
            "b1": _w((lambda *s: _rng.normal(s) * 0.05)(F)),
            "w2": _w((lambda *s: _rng.normal(s) * 0.05)(F, D) * (F ** -0.5)),
        }
    _B_in = _B_setup()

    return {
        "A_x": _A_in["x"],
        "A_wqkv": _A_in["wqkv"],
        "A_wo": _A_in["wo"],
        "B_x": _B_in["x"],
        "B_w1": _B_in["w1"],
        "B_b1": _B_in["b1"],
        "B_w2": _B_in["w2"],
    }

def reference(A_x, A_wqkv, A_wo, B_x, B_w1, B_b1, B_w2):
    def _A_ref(x, wqkv, wo):
        B, S, D = x.shape
        H = 32
        Dh = D // H
        qkv = (lambda x, *d: x.transpose(*d))((x @ wqkv).reshape(B, S, 3, H, Dh), 2, 0, 3, 1, 4)
        q, k, v = qkv[0], qkv[1], qkv[2]
        scores = jnp.einsum("bhqd,bhkd->bhqk", q, k) * (Dh ** -0.5)
        p = _softmax(scores, axis=-1)
        o = jnp.einsum("bhqk,bhkd->bhqd", p, v)
        return (lambda x, *d: x.transpose(*d))(o, 0, 2, 1, 3).reshape(B, S, D) @ wo

    def _B_ref(x, w1, b1, w2):
        h = jnp.einsum("bsd,df->bsf", x, w1) + b1
        sp = jnp.log1p(jnp.exp(-jnp.abs(h))) + jnp.where(h > 0, h, jnp.zeros_like(h))
        act = h * jnp.tanh(sp)
        return jnp.einsum("bsf,fd->bsd", act, w2)

    x = A_x
    h = x + _A_ref(_layernorm(x, axis=-1), A_wqkv, A_wo)
    h2 = h + _B_ref(_layernorm(h, axis=-1), B_w1, B_b1, B_w2)
    return h2
```

```python
import functools
import math

import jax
import jax.numpy as jnp
from jax import lax
import jax.experimental.pallas as pl
import jax.experimental.pallas.tpu as pltpu

S = 2048
D = 576
H = 32
DH = 18
F = 4608
BQ = 512
NB = S // BQ
KC = 128
NCH = S // KC
HPG = 7
NG = 5
MV = 24
UH = 8
FC = 2304
EPS = 1e-5
QSCALE = float(DH ** -0.5 * math.log2(math.e))

f32 = jnp.float32
bf16 = jnp.bfloat16


def _tn(a, b):
    return lax.dot_general(a, b, (((0,), (0,)), ((), ())), preferred_element_type=f32)


def _pad_heads_lanes(w):
    rows = w.shape[0]
    parts = []
    for g in range(NG):
        lo = g * HPG * DH
        hi = min(lo + HPG * DH, D)
        parts.append(w[:, lo:hi])
        parts.append(jnp.zeros((rows, 128 - (hi - lo)), w.dtype))
    return jnp.concatenate(parts, axis=1)


def _ln_t(xt):
    m = jnp.sum(xt, axis=0, keepdims=True) * (1.0 / D)
    d = xt - m
    v = jnp.sum(d * d, axis=0, keepdims=True) * (1.0 / D)
    return d * lax.rsqrt(v + EPS)


def kernel(x_hbm, wqkv_hbm, wo_hbm, w1_hbm, b1_ref, w2_hbm, out_ref,
           x_ref, wqkv_ref, wo_ref, w2_ref,
           k_ref, qm_ref, vt_ref, s_ref, m_ref, ot_ref, w1a_ref, wq_ref, wk_ref, hn_ref, acc_ref, sem):
    blk = pl.program_id(0)

    def cp_x(t):
        return pltpu.make_async_copy(x_hbm.at[:, pl.ds(t * BQ, BQ)], x_ref.at[t], sem.at[t])

    cp_wqkv = pltpu.make_async_copy(wqkv_hbm, wqkv_ref, sem.at[NB])
    cp_wo = pltpu.make_async_copy(wo_hbm, wo_ref, sem.at[NB + 1])
    cp_w1 = pltpu.make_async_copy(w1_hbm, w1a_ref.at[0:D], sem.at[NB + 2])
    cp_w2 = pltpu.make_async_copy(w2_hbm, w2_ref, sem.at[NB + 3])

    def step(np_, slot_p, nc, slot_c, mc):
        g = (np_ % H) // HPG
        mp = None
        acc = None
        for j in range(NCH):
            sl = slice(j * KC, (j + 1) * KC)
            s = jnp.dot(k_ref[g, sl, :], qm_ref[np_], preferred_element_type=f32)
            s_ref[slot_p, sl, :] = s
            sm = jnp.max(s.reshape(KC // 8, 8, BQ), axis=0)
            mp = sm if mp is None else jnp.maximum(mp, sm)
            if nc is not None:
                p = jnp.exp2(s_ref[slot_c, sl, :] - mc).astype(bf16)
                d = jnp.dot(vt_ref[nc % H, :, sl], p, preferred_element_type=f32)
                acc = d if acc is None else acc + d
        o = None
        if nc is not None:
            o = acc[0:DH] * (1.0 / acc[DH:DH + 1])
        return jnp.max(mp, axis=0, keepdims=True), o

    @pl.when(blk == 0)
    def _prologue():
        cp_wqkv.start()
        cp_x(0).start()
        brow = jnp.concatenate([b1_ref[...].astype(f32).reshape(1, F), jnp.zeros((15, F), f32)], axis=0)
        w1a_ref[D:D + 16, :] = brow.astype(bf16)
        cp_wqkv.wait()
        for t in range(1, NB):
            cp_x(t).start()
        cp_wo.start()
        cp_w1.start()
        cp_w2.start()
        wq_ref[...] = _pad_heads_lanes(wqkv_ref[:, 0:D].astype(f32)).astype(bf16)
        wk_ref[...] = _pad_heads_lanes(wqkv_ref[:, D:2 * D].astype(f32)).astype(bf16)
        row = lax.broadcasted_iota(jnp.int32, (128, BQ), 0)

        def pbody(t, _):
            tok = pl.ds(pl.multiple_of(t * BQ, BQ), BQ)
            cp_x(t).wait()
            xt = x_ref[t].astype(f32)
            xn = _ln_t(xt).astype(bf16)
            qt = _tn(wq_ref[...], xn) * QSCALE
            for h in range(H):
                g, lo = h // HPG, (h % HPG) * DH
                qm_ref[t * H + h] = jnp.where((row >= lo) & (row < lo + DH), qt[g * 128:(g + 1) * 128], 0.0).astype(bf16)
            kk = _tn(xn, wk_ref[...]).astype(bf16)
            for g in range(NG):
                k_ref[g, tok, :] = kk[:, g * 128:(g + 1) * 128]
            vt = _tn(wqkv_ref[:, 2 * D:3 * D], xn).astype(bf16).astype(f32)
            tail = jnp.concatenate([jnp.ones((1, BQ), f32), jnp.zeros((MV - DH - 1, BQ), f32)], axis=0)
            for h in range(H):
                vt_ref[h, :, tok] = jnp.concatenate([vt[h * DH:(h + 1) * DH], tail], axis=0)
            return _

        lax.fori_loop(0, NB, pbody, None)
        m0, _ = step(0, 0, None, None, None)
        m_ref[...] = m0

    def body(i, m):
        og = ot_ref.at[pl.ds(pl.multiple_of(i * UH * DH, 8), UH * DH), :]
        for u in range(UH):
            nc = blk * H + UH * i + u
            np_ = jnp.minimum(nc + 1, NB * H - 1)
            m, o = step(np_, (u + 1) % 2, nc, u % 2, m)
            og[u * DH:(u + 1) * DH, :] = o
        return m

    m_ref[...] = lax.fori_loop(0, H // UH, body, m_ref[...])

    @pl.when(blk == 0)
    def _wait_weights():
        cp_wo.wait()
        cp_w1.wait()
        cp_w2.wait()

    ot = ot_ref[...].astype(bf16)
    ht = x_ref[blk].astype(f32) + _tn(wo_ref[...], ot)
    acc_ref[...] = ht
    hn_ref[0:D, :] = _ln_t(ht).astype(bf16)
    hn_ref[D:D + 16, :] = jnp.concatenate([jnp.ones((1, BQ), f32), jnp.zeros((15, BQ), f32)], axis=0).astype(bf16)

    def fbody(c, _):
        fs = pl.ds(pl.multiple_of(c * FC, 128), FC)
        z = _tn(w1a_ref[:, fs], hn_ref[...])
        sp = jnp.log1p(jnp.exp(-jnp.abs(z))) + jnp.maximum(z, 0.0)
        act = (z * jnp.tanh(sp)).astype(bf16)
        acc_ref[...] += jnp.dot(w2_ref[:, fs], act, preferred_element_type=f32)
        return _

    lax.fori_loop(0, F // FC, fbody, None)
    out_ref[...] = acc_ref[...].astype(bf16)


@jax.jit
def pallas_sequential_preLN__mha_block__dense_activation_mish__prompt_kernel(
    A_x, A_wqkv, A_wo, B_x, B_w1, B_b1, B_w2,
):
    del B_x
    x2 = A_x.reshape(S, D).T
    hbm = pl.BlockSpec(memory_space=pltpu.HBM)
    out = pl.pallas_call(
        kernel,
        grid=(NB,),
        in_specs=[hbm, hbm, hbm, hbm, pl.BlockSpec((F,), lambda i: (0,)), hbm],
        out_specs=pl.BlockSpec((D, BQ), lambda i: (0, i)),
        out_shape=jax.ShapeDtypeStruct((D, S), bf16),
        scratch_shapes=[
            pltpu.VMEM((NB, D, BQ), bf16),
            pltpu.VMEM((D, 3 * D), bf16),
            pltpu.VMEM((D, D), bf16),
            pltpu.VMEM((D, F), bf16),
            pltpu.VMEM((NG, S, 128), bf16),
            pltpu.VMEM((NB * H, 128, BQ), bf16),
            pltpu.VMEM((H, MV, S), f32),
            pltpu.VMEM((2, S, BQ), f32),
            pltpu.VMEM((1, BQ), f32),
            pltpu.VMEM((D, BQ), f32),
            pltpu.VMEM((D + 16, F), bf16),
            pltpu.VMEM((D, NG * 128), bf16),
            pltpu.VMEM((D, NG * 128), bf16),
            pltpu.VMEM((D + 16, BQ), bf16),
            pltpu.VMEM((D, BQ), f32),
            pltpu.SemaphoreType.DMA((NB + 4,)),
        ],
        compiler_params=pltpu.CompilerParams(
            dimension_semantics=("arbitrary",),
            vmem_limit_bytes=100 * 1024 * 1024,
        ),
    )(x2, A_wqkv, A_wo, B_w1, B_b1, B_w2.T)
    return out.T.reshape(1, S, D)
```

```python
import math

import jax
import jax.numpy as jnp
from jax import lax
import jax.experimental.pallas as pl
import jax.experimental.pallas.tpu as pltpu

S = 2048
D = 576
H = 32
DH = D // H
F = 4608
EPS = 1e-5

BQ = 512
NB = S // BQ
KC = 128
NCH = S // KC
HPG = 4
NG = H // HPG
MV = 24
LAG = 2
UH = 8
FC = 2304
HF = FC // 2
HM = D // 2
HT = BQ // 2
FQ = F // NB
RQ = D // 4
DA = D + 16

QSCALE = float(DH ** -0.5 * math.log2(math.e))

f32 = jnp.float32
bf16 = jnp.bfloat16


def _dot(a, b):
    return jnp.dot(a, b, preferred_element_type=f32)


def _dot_tn(a, b):
    return lax.dot_general(a, b, (((0,), (0,)), ((), ())), preferred_element_type=f32)


def _layernorm_t(xt):
    m = jnp.sum(xt, axis=0, keepdims=True) * (1.0 / D)
    d = xt - m
    v = jnp.sum(d * d, axis=0, keepdims=True) * (1.0 / D)
    return d * lax.rsqrt(v + EPS)


def _mish(z):
    sp = jnp.log1p(jnp.exp(-jnp.abs(z))) + jnp.maximum(z, 0.0)
    return z * jnp.tanh(sp)


def _kernel(x_hbm, wqkv_hbm, wo_hbm, w1_hbm, b1_hbm, w2_hbm, out_ref,
            x_ref, wqkv_ref, wo_ref, w2_ref, k_ref, q_ref, vt_ref, s_ref,
            m_ref, mp_ref, ot_ref, w1_ref, hn_ref, acc_ref, xn_ref, w1t_ref,
            wot_ref, b1_ref, brow_ref, ws_ref, sem):
    blk = pl.program_id(0)

    def cp_x(t):
        return pltpu.make_async_copy(x_hbm.at[:, pl.ds(t * BQ, BQ)], x_ref.at[t], sem.at[t])

    def cp_w1(t):
        cols = pl.ds(t * FQ, FQ)
        return pltpu.make_async_copy(w1_hbm.at[:, cols], w1_ref.at[:, cols], sem.at[NB + t])

    def cp_w2(t, half):
        rows = pl.ds(half * HM + (t % 2) * RQ, RQ)
        cols = pl.ds((t // 2) * FC, FC)
        return pltpu.make_async_copy(w2_hbm.at[rows, cols], w2_ref.at[rows, cols],
                                     sem.at[2 * NB + 2 * t + half])

    cp_wqk = pltpu.make_async_copy(wqkv_hbm.at[:, 0:2 * D], wqkv_ref.at[:, 0:2 * D], sem.at[4 * NB])
    cp_wv = pltpu.make_async_copy(wqkv_hbm.at[:, 2 * D:3 * D], wqkv_ref.at[:, 2 * D:3 * D],
                                  sem.at[4 * NB + 1])
    cp_wo = pltpu.make_async_copy(wo_hbm, wo_ref, sem.at[4 * NB + 2])
    cp_b1 = pltpu.make_async_copy(b1_hbm, b1_ref.at[0:F], sem.at[4 * NB + 3])

    def produce(n, pos, slot, j, mp):
        g = (n % H) // HPG
        keys = slice(j * KC, (j + 1) * KC)
        rows = [q_ref[n], jnp.zeros((128 - 32 - 16 * pos, BQ), bf16)]
        if pos:
            rows.insert(0, jnp.zeros((16 * pos, BQ), bf16))
        s = _dot(k_ref[g, keys, :], jnp.concatenate(rows, axis=0))
        s_ref[slot, keys, :] = s
        sm = jnp.max(s.reshape(KC // 8, 8, BQ), axis=0)
        return sm if mp is None else jnp.maximum(mp, sm)

    def consume(n, slot, j, m, acc):
        keys = slice(j * KC, (j + 1) * KC)
        p = jnp.exp2(s_ref[slot, keys, :] - m).astype(bf16)
        d = _dot(vt_ref[n % H, :, keys], p)
        return d if acc is None else acc + d

    def step(n, u, m, mp):
        par = u % 2
        n1 = jnp.minimum(n + 1, NB * H - 1)
        n2 = jnp.minimum(n + 2, NB * H - 1)
        acc = None
        m_next = None
        for j in range(NCH):
            jp = j + LAG
            if jp < NCH:
                mp = produce(n1, (u + 1) % HPG, 1 - par, jp, mp)
                if jp == NCH - 1:
                    m_next = jnp.max(mp, axis=0, keepdims=True)
                    mp = None
            else:
                mp = produce(n2, (u + 2) % HPG, par, jp - NCH, mp)
            acc = consume(n, par, j, m, acc)
        o = acc[0:DH] * (1.0 / acc[DH:DH + 1])
        return m_next, mp, o

    @pl.when(blk == 0)
    def _prologue():
        cp_x(0).start()
        cp_wv.start()
        cp_b1.start()
        cp_wv.wait()
        for t in range(1, NB):
            cp_x(t).start()

        def v_body(t, _):
            tok = pl.ds(pl.multiple_of(t * BQ, BQ), BQ)
            cp_x(t).wait()

            @pl.when(t == 0)
            def _():
                cp_wqk.start()
                for tt in range(NB):
                    cp_w1(tt).start()
                    cp_w2(tt, 0).start()
                    cp_w2(tt, 1).start()
                cp_wo.start()

            xn = _layernorm_t(x_ref[t].astype(f32)).astype(bf16)
            xn_ref[t] = xn
            vt = _dot_tn(wqkv_ref[:, 2 * D:3 * D], xn).astype(bf16).astype(f32)
            tail = jnp.concatenate([jnp.ones((1, BQ), f32), jnp.zeros((MV - DH - 1, BQ), f32)], axis=0)
            for h in range(H):
                vt_ref[h, :, tok] = jnp.concatenate([vt[h * DH:(h + 1) * DH], tail], axis=0)
            return _

        lax.fori_loop(0, NB, v_body, None)
        cp_b1.wait()
        brow_ref[...] = jnp.concatenate(
            [b1_ref[0:F].astype(f32).reshape(1, F), jnp.zeros((DA - D - 1, F), f32)], axis=0).astype(bf16)
        cp_wqk.wait()
        row = lax.broadcasted_iota(jnp.int32, (32, BQ), 0)

        def qk_body(t, _):
            tok = pl.ds(pl.multiple_of(t * BQ, BQ), BQ)
            cp_w1(t).wait()
            cp_w2(t, 0).wait()
            cp_w2(t, 1).wait()
            xn = xn_ref[t]
            QS = 512
            hi_part = _dot_tn(wqkv_ref[:, QS:2 * D], xn)
            for g in range(NG):
                lo = D + g * HPG * DH - QS
                hi = min(lo + 128, 2 * D - QS)
                kg = hi_part[lo:hi]
                if hi - lo < 128:
                    kg = jnp.concatenate([kg, jnp.zeros((128 - (hi - lo), BQ), f32)], axis=0)
                k_ref[g, tok, :] = kg.astype(bf16).T
            q = jnp.concatenate([_dot_tn(wqkv_ref[:, 0:QS], xn), hi_part[0:D + 32 - QS]], axis=0)
            for h in range(H):
                j = h % HPG
                src = (h // HPG) * HPG * DH + 16 * j
                q_ref[t * H + h] = jnp.where(
                    (row >= 2 * j) & (row < 2 * j + DH), q[src:src + 32] * QSCALE, 0.0).astype(bf16)
            fq = pl.ds(pl.multiple_of(t * FQ, 128), FQ)
            w1t_ref[fq, :] = jnp.concatenate([w1_ref[:, fq], brow_ref[:, fq]], axis=0).T
            c = t // 2
            for rg in range(RQ // 16):
                top = pl.ds(pl.multiple_of((t % 2) * RQ + rg * 16, 16), 16)
                bot = pl.ds(pl.multiple_of(HM + (t % 2) * RQ + rg * 16, 16), 16)
                for lg in range(HF // 384):
                    l1 = pl.ds(pl.multiple_of(c * FC + lg * 384, 128), 384)
                    l2 = pl.ds(pl.multiple_of(c * FC + HF + lg * 384, 128), 384)
                    a11, a12 = w2_ref[top, l1].astype(f32), w2_ref[top, l2].astype(f32)
                    a21, a22 = w2_ref[bot, l1].astype(f32), w2_ref[bot, l2].astype(f32)
                    dst = slice(lg * 384, (lg + 1) * 384)
                    ws_ref[c, 0, top, dst] = (a11 + a22).astype(bf16)
                    ws_ref[c, 1, top, dst] = (a21 + a22).astype(bf16)
                    ws_ref[c, 2, top, dst] = (a11 + a12).astype(bf16)
                    ws_ref[c, 3, top, dst] = (a21 - a11).astype(bf16)
                    ws_ref[c, 4, top, dst] = (a12 - a22).astype(bf16)
            return _

        lax.fori_loop(0, NB, qk_body, None)
        cp_wo.wait()
        wot_ref[...] = wo_ref[...].T
        mp = None
        for j in range(NCH):
            mp = produce(0, 0, 0, j, mp)
        m_ref[0:1, :] = jnp.max(mp, axis=0, keepdims=True)
        mp = None
        for j in range(LAG):
            mp = produce(1, 1, 1, j, mp)
        mp_ref[...] = mp

    def att_body(i, carry):
        m, mp = carry
        og = ot_ref.at[pl.ds(pl.multiple_of(i * UH * DH, 8), UH * DH), :]
        for u in range(UH):
            m, mp, o = step(blk * H + UH * i + u, u, m, mp)
            og[u * DH:(u + 1) * DH, :] = o
        return m, mp

    m_ref[0:1, :], mp_ref[...] = lax.fori_loop(0, H // UH, att_body, (m_ref[0:1, :], mp_ref[...]))

    ht = x_ref[blk].astype(f32) + _dot(wot_ref[...], ot_ref[...].astype(bf16))
    acc_ref[...] = ht
    hn_ref[0:D, :] = _layernorm_t(ht).astype(bf16)
    hn_ref[D:DA, :] = jnp.concatenate(
        [jnp.ones((1, BQ), f32), jnp.zeros((DA - D - 1, BQ), f32)], axis=0).astype(bf16)

    def ffn_body(c, _):
        fs = pl.ds(pl.multiple_of(c * FC, 128), FC)
        act = _mish(_dot(w1t_ref[fs, :], hn_ref[...]))
        b11, b12 = act[0:HF, 0:HT], act[0:HF, HT:]
        b21, b22 = act[HF:, 0:HT], act[HF:, HT:]
        f1 = pl.ds(pl.multiple_of(c * FC, 128), HF)
        f2 = pl.ds(pl.multiple_of(c * FC + HF, 128), HF)
        mm = lambda a, b: _dot(a, b.astype(bf16))
        m2 = mm(ws_ref[c, 1], b11)
        m6 = mm(ws_ref[c, 3], b11 + b12)
        m5 = mm(ws_ref[c, 2], b22)
        m1 = mm(ws_ref[c, 0], b11 + b22)
        m3 = mm(w2_ref[0:HM, f1], b12 - b22)
        m4 = mm(w2_ref[HM:, f2], b21 - b11)
        m7 = mm(ws_ref[c, 4], b21 + b22)
        top, bot, left, right = slice(0, HM), slice(HM, D), slice(0, HT), slice(HT, BQ)
        for rows, cols, d in ((top, left, (m1 + m4) + (m7 - m5)), (top, right, m3 + m5),
                              (bot, left, m2 + m4), (bot, right, (m1 - m2) + (m3 + m6))):
            v = acc_ref[rows, cols] + d
            acc_ref[rows, cols] = v
            out_ref[rows, cols] = v.astype(bf16)
        return _

    lax.fori_loop(0, F // FC, ffn_body, None)


@jax.jit
def pallas_sequential_preLN__mha_block__dense_activation_mish__prompt_kernel(
    A_x: jax.Array,
    A_wqkv: jax.Array,
    A_wo: jax.Array,
    B_x: jax.Array,
    B_w1: jax.Array,
    B_b1: jax.Array,
    B_w2: jax.Array,
):
    del B_x
    hbm = pl.BlockSpec(memory_space=pltpu.HBM)
    out_t = pl.pallas_call(
        _kernel,
        grid=(NB,),
        in_specs=[hbm] * 6,
        out_specs=pl.BlockSpec((D, BQ), lambda i: (0, i)),
        out_shape=jax.ShapeDtypeStruct((D, S), bf16),
        scratch_shapes=[
            pltpu.VMEM((NB, D, BQ), bf16),
            pltpu.VMEM((D, 3 * D), bf16),
            pltpu.VMEM((D, D), bf16),
            pltpu.VMEM((D, F), bf16),
            pltpu.VMEM((NG, S, 128), bf16),
            pltpu.VMEM((NB * H, 32, BQ), bf16),
            pltpu.VMEM((H, MV, S), f32),
            pltpu.VMEM((2, S, BQ), f32),
            pltpu.VMEM((8, BQ), f32),
            pltpu.VMEM((8, BQ), f32),
            pltpu.VMEM((D, BQ), f32),
            pltpu.VMEM((D, F), bf16),
            pltpu.VMEM((DA, BQ), bf16),
            pltpu.VMEM((D, BQ), f32),
            pltpu.VMEM((NB, D, BQ), bf16),
            pltpu.VMEM((F, DA), bf16),
            pltpu.VMEM((D, D), bf16),
            pltpu.VMEM((F + 1536,), bf16),
            pltpu.VMEM((DA - D, F), bf16),
            pltpu.VMEM((F // FC, 5, HM, HF), bf16),
            pltpu.SemaphoreType.DMA((4 * NB + 4,)),
        ],
        compiler_params=pltpu.CompilerParams(
            dimension_semantics=("arbitrary",),
            vmem_limit_bytes=100 * 1024 * 1024,
        ),
    )(A_x.reshape(S, D).T, A_wqkv, A_wo, B_w1, B_b1, B_w2.T)
    return out_t.T.reshape(1, S, D)
```

```python
import math

import jax
import jax.numpy as jnp
from jax import lax
import jax.experimental.pallas as pl
import jax.experimental.pallas.tpu as pltpu

S = 2048
D = 576
H = 32
DH = D // H
F = 4608
EPS = 1e-5

BQ = 512
NB = S // BQ
KC = 128
NCH = S // KC
HPG = 4
NG = H // HPG
MV = 24
LAG = 1
UH = 8
FC = 2304
HF = FC // 2
HM = D // 2
HT = BQ // 2
FQ = F // NB
RQ = D // 4
DA = D + 16

QSCALE = float(DH ** -0.5 * math.log2(math.e))

f32 = jnp.float32
bf16 = jnp.bfloat16


def _dot(a, b):
    return jnp.dot(a, b, preferred_element_type=f32)


def _dot_tn(a, b):
    return lax.dot_general(a, b, (((0,), (0,)), ((), ())), preferred_element_type=f32)


def _layernorm_t(xt):
    m = jnp.sum(xt, axis=0, keepdims=True) * (1.0 / D)
    d = xt - m
    v = jnp.sum(d * d, axis=0, keepdims=True) * (1.0 / D)
    return d * lax.rsqrt(v + EPS)


def _mish(z):
    sp = jnp.log1p(jnp.exp(-jnp.abs(z))) + jnp.maximum(z, 0.0)
    return z * jnp.tanh(sp)


def _kernel(x_hbm, wqkv_hbm, wo_hbm, w1_hbm, b1_hbm, w2_hbm, out_ref,
            x_ref, wqkv_ref, wo_ref, w2_ref, k_ref, q_ref, vt_ref, s_ref,
            m_ref, mp_ref, ot_ref, w1_ref, hn_ref, acc_ref, xn_ref, w1t_ref,
            wot_ref, b1_ref, brow_ref, ws_ref, rs_ref, sem):
    blk = pl.program_id(0)

    def cp_x(t):
        return pltpu.make_async_copy(x_hbm.at[:, pl.ds(t * BQ, BQ)], x_ref.at[t], sem.at[t])

    def cp_w1(t):
        cols = pl.ds(t * FQ, FQ)
        return pltpu.make_async_copy(w1_hbm.at[:, cols], w1_ref.at[:, cols], sem.at[NB + t])

    def cp_w2(t, half):
        rows = pl.ds(half * HM + (t % 2) * RQ, RQ)
        cols = pl.ds((t // 2) * FC, FC)
        return pltpu.make_async_copy(w2_hbm.at[rows, cols], w2_ref.at[rows, cols],
                                     sem.at[2 * NB + 2 * t + half])

    cp_wqk = pltpu.make_async_copy(wqkv_hbm.at[:, 0:2 * D], wqkv_ref.at[:, 0:2 * D], sem.at[4 * NB])
    cp_wv = pltpu.make_async_copy(wqkv_hbm.at[:, 2 * D:3 * D], wqkv_ref.at[:, 2 * D:3 * D],
                                  sem.at[4 * NB + 1])
    cp_wo = pltpu.make_async_copy(wo_hbm, wo_ref, sem.at[4 * NB + 2])
    cp_b1 = pltpu.make_async_copy(b1_hbm, b1_ref.at[0:F], sem.at[4 * NB + 3])

    def produce(n, pos, slot, j, mp):
        g = (n % H) // HPG
        keys = slice(j * KC, (j + 1) * KC)
        rows = [q_ref[n], jnp.zeros((128 - 32 - 16 * pos, BQ), bf16)]
        if pos:
            rows.insert(0, jnp.zeros((16 * pos, BQ), bf16))
        s = _dot(k_ref[g, keys, :], jnp.concatenate(rows, axis=0))
        s_ref[slot, keys, :] = s
        sm = jnp.max(s.reshape(KC // 8, 8, BQ), axis=0)
        return sm if mp is None else jnp.maximum(mp, sm)

    def consume(n, slot, j, m, acc):
        keys = slice(j * KC, (j + 1) * KC)
        p = jnp.exp2(s_ref[slot, keys, :] - m).astype(bf16)
        d = _dot(vt_ref[n % H, :, keys], p)
        return d if acc is None else acc + d

    def step(n, u, m, mp):
        par = u % 2
        n1 = jnp.minimum(n + 1, NB * H - 1)
        n2 = jnp.minimum(n + 2, NB * H - 1)
        acc = None
        m_next = None
        for j in range(NCH):
            jp = j + LAG
            if jp < NCH:
                mp = produce(n1, (u + 1) % HPG, 1 - par, jp, mp)
                if jp == NCH - 1:
                    m_next = jnp.max(mp, axis=0, keepdims=True)
                    mp = None
            else:
                mp = produce(n2, (u + 2) % HPG, par, jp - NCH, mp)
            acc = consume(n, par, j, m, acc)
        o = acc[0:DH] * (1.0 / acc[DH:DH + 1])
        return m_next, mp, o

    @pl.when(blk == 0)
    def _prologue():
        cp_x(0).start()
        cp_wv.start()
        cp_b1.start()
        cp_wv.wait()
        for t in range(1, NB):
            cp_x(t).start()

        def v_body(t, _):
            tok = pl.ds(pl.multiple_of(t * BQ, BQ), BQ)
            cp_x(t).wait()

            @pl.when(t == 0)
            def _():
                cp_wqk.start()
                for tt in range(NB):
                    cp_w1(tt).start()
                    cp_w2(tt, 0).start()
                    cp_w2(tt, 1).start()
                cp_wo.start()

            xt = x_ref[t].astype(f32)
            xc = xt - jnp.sum(xt, axis=0, keepdims=True) * (1.0 / D)
            rs = lax.rsqrt(jnp.sum(xc * xc, axis=0, keepdims=True) * (1.0 / D) + EPS)
            xn = xc.astype(bf16)
            xn_ref[t] = xn
            rs_ref[t, 0:1, :] = rs
            vt = (_dot_tn(wqkv_ref[:, 2 * D:3 * D], xn) * rs).astype(bf16).astype(f32)
            tail = jnp.concatenate([jnp.ones((1, BQ), f32), jnp.zeros((MV - DH - 1, BQ), f32)], axis=0)
            for h in range(H):
                vt_ref[h, :, tok] = jnp.concatenate([vt[h * DH:(h + 1) * DH], tail], axis=0)
            return _

        lax.fori_loop(0, NB, v_body, None)
        cp_b1.wait()
        brow_ref[...] = jnp.concatenate(
            [b1_ref[0:F].astype(f32).reshape(1, F), jnp.zeros((DA - D - 1, F), f32)], axis=0).astype(bf16)
        cp_wqk.wait()
        row = lax.broadcasted_iota(jnp.int32, (32, BQ), 0)

        def qk_body(t, _):
            tok = pl.ds(pl.multiple_of(t * BQ, BQ), BQ)
            cp_w1(t).wait()
            cp_w2(t, 0).wait()
            cp_w2(t, 1).wait()
            xn = xn_ref[t]
            rs = rs_ref[t, 0:1, :]
            QS = 512
            hi_part = _dot_tn(wqkv_ref[:, QS:2 * D], xn) * rs
            for g in range(NG):
                lo = D + g * HPG * DH - QS
                hi = min(lo + 128, 2 * D - QS)
                kg = hi_part[lo:hi]
                if hi - lo < 128:
                    kg = jnp.concatenate([kg, jnp.zeros((128 - (hi - lo), BQ), f32)], axis=0)
                k_ref[g, tok, :] = kg.astype(bf16).T
            q = jnp.concatenate([_dot_tn(wqkv_ref[:, 0:QS], xn) * rs, hi_part[0:D + 32 - QS]], axis=0)
            for h in range(H):
                j = h % HPG
                src = (h // HPG) * HPG * DH + 16 * j
                q_ref[t * H + h] = jnp.where(
                    (row >= 2 * j) & (row < 2 * j + DH), q[src:src + 32] * QSCALE, 0.0).astype(bf16)
            fq = pl.ds(pl.multiple_of(t * FQ, 128), FQ)
            w1t_ref[fq, :] = jnp.concatenate([w1_ref[:, fq], brow_ref[:, fq]], axis=0).T
            c = t // 2
            for rg in range(RQ // 16):
                top = pl.ds(pl.multiple_of((t % 2) * RQ + rg * 16, 16), 16)
                bot = pl.ds(pl.multiple_of(HM + (t % 2) * RQ + rg * 16, 16), 16)
                for lg in range(HF // 384):
                    l1 = pl.ds(pl.multiple_of(c * FC + lg * 384, 128), 384)
                    l2 = pl.ds(pl.multiple_of(c * FC + HF + lg * 384, 128), 384)
                    a11, a12 = w2_ref[top, l1].astype(f32), w2_ref[top, l2].astype(f32)
                    a21, a22 = w2_ref[bot, l1].astype(f32), w2_ref[bot, l2].astype(f32)
                    dst = slice(lg * 384, (lg + 1) * 384)
                    ws_ref[c, 0, top, dst] = (a11 + a22).astype(bf16)
                    ws_ref[c, 1, top, dst] = (a21 + a22).astype(bf16)
                    ws_ref[c, 2, top, dst] = (a11 + a12).astype(bf16)
                    ws_ref[c, 3, top, dst] = (a21 - a11).astype(bf16)
                    ws_ref[c, 4, top, dst] = (a12 - a22).astype(bf16)
            return _

        lax.fori_loop(0, NB, qk_body, None)
        cp_wo.wait()
        wot_ref[...] = wo_ref[...].T
        mp = None
        for j in range(NCH):
            mp = produce(0, 0, 0, j, mp)
        m_ref[0:1, :] = jnp.max(mp, axis=0, keepdims=True)
        mp = None
        for j in range(LAG):
            mp = produce(1, 1, 1, j, mp)
        mp_ref[...] = mp

    def att_body(i, carry):
        m, mp = carry
        og = ot_ref.at[pl.ds(pl.multiple_of(i * UH * DH, 8), UH * DH), :]
        for u in range(UH):
            m, mp, o = step(blk * H + UH * i + u, u, m, mp)
            og[u * DH:(u + 1) * DH, :] = o
        return m, mp

    m_ref[0:1, :], mp_ref[...] = lax.fori_loop(0, H // UH, att_body, (m_ref[0:1, :], mp_ref[...]))

    ht = x_ref[blk].astype(f32) + _dot(wot_ref[...], ot_ref[...].astype(bf16))
    acc_ref[...] = ht
    hn_ref[0:D, :] = _layernorm_t(ht).astype(bf16)
    hn_ref[D:DA, :] = jnp.concatenate(
        [jnp.ones((1, BQ), f32), jnp.zeros((DA - D - 1, BQ), f32)], axis=0).astype(bf16)

    def ffn_body(c, _):
        fs = pl.ds(pl.multiple_of(c * FC, 128), FC)
        act = _mish(_dot(w1t_ref[fs, :], hn_ref[...]))
        b11, b12 = act[0:HF, 0:HT], act[0:HF, HT:]
        b21, b22 = act[HF:, 0:HT], act[HF:, HT:]
        f1 = pl.ds(pl.multiple_of(c * FC, 128), HF)
        f2 = pl.ds(pl.multiple_of(c * FC + HF, 128), HF)
        mm = lambda a, b: _dot(a, b.astype(bf16))
        m2 = mm(ws_ref[c, 1], b11)
        m6 = mm(ws_ref[c, 3], b11 + b12)
        m5 = mm(ws_ref[c, 2], b22)
        m1 = mm(ws_ref[c, 0], b11 + b22)
        m3 = mm(w2_ref[0:HM, f1], b12 - b22)
        m4 = mm(w2_ref[HM:, f2], b21 - b11)
        m7 = mm(ws_ref[c, 4], b21 + b22)
        top, bot, left, right = slice(0, HM), slice(HM, D), slice(0, HT), slice(HT, BQ)
        for rows, cols, d in ((top, left, (m1 + m4) + (m7 - m5)), (top, right, m3 + m5),
                              (bot, left, m2 + m4), (bot, right, (m1 - m2) + (m3 + m6))):
            v = acc_ref[rows, cols] + d
            acc_ref[rows, cols] = v
            out_ref[rows, cols] = v.astype(bf16)
        return _

    lax.fori_loop(0, F // FC, ffn_body, None)


@jax.jit
def pallas_sequential_preLN__mha_block__dense_activation_mish__prompt_kernel(
    A_x: jax.Array,
    A_wqkv: jax.Array,
    A_wo: jax.Array,
    B_x: jax.Array,
    B_w1: jax.Array,
    B_b1: jax.Array,
    B_w2: jax.Array,
):
    del B_x
    hbm = pl.BlockSpec(memory_space=pltpu.HBM)
    out_t = pl.pallas_call(
        _kernel,
        grid=(NB,),
        in_specs=[hbm] * 6,
        out_specs=pl.BlockSpec((D, BQ), lambda i: (0, i)),
        out_shape=jax.ShapeDtypeStruct((D, S), bf16),
        scratch_shapes=[
            pltpu.VMEM((NB, D, BQ), bf16),
            pltpu.VMEM((D, 3 * D), bf16),
            pltpu.VMEM((D, D), bf16),
            pltpu.VMEM((D, F), bf16),
            pltpu.VMEM((NG, S, 128), bf16),
            pltpu.VMEM((NB * H, 32, BQ), bf16),
            pltpu.VMEM((H, MV, S), f32),
            pltpu.VMEM((2, S, BQ), f32),
            pltpu.VMEM((8, BQ), f32),
            pltpu.VMEM((8, BQ), f32),
            pltpu.VMEM((D, BQ), f32),
            pltpu.VMEM((D, F), bf16),
            pltpu.VMEM((DA, BQ), bf16),
            pltpu.VMEM((D, BQ), f32),
            pltpu.VMEM((NB, D, BQ), bf16),
            pltpu.VMEM((F, DA), bf16),
            pltpu.VMEM((D, D), bf16),
            pltpu.VMEM((F + 1536,), bf16),
            pltpu.VMEM((DA - D, F), bf16),
            pltpu.VMEM((F // FC, 5, HM, HF), bf16),
            pltpu.VMEM((NB, 8, BQ), f32),
            pltpu.SemaphoreType.DMA((4 * NB + 4,)),
        ],
        compiler_params=pltpu.CompilerParams(
            dimension_semantics=("arbitrary",),
            vmem_limit_bytes=100 * 1024 * 1024,
        ),
    )(A_x.reshape(S, D).T, A_wqkv, A_wo, B_w1, B_b1, B_w2.T)
    return out_t.T.reshape(1, S, D)
```

```python
import math

import jax
import jax.numpy as jnp
from jax import lax
import jax.experimental.pallas as pl
import jax.experimental.pallas.tpu as pltpu

S = 2048
D = 576
H = 32
DH = D // H
F = 4608
EPS = 1e-5

BQ = 512
NB = S // BQ
KC = 128
NCH = S // KC
HPG = 4
NG = H // HPG
MV = 24
LAG = 1
UH = 8
FC = 2304
HF = FC // 2
HM = D // 2
HT = BQ // 2
FQ = F // NB
RQ = D // 4
DA = D + 16

QSCALE = float(DH ** -0.5 * math.log2(math.e))

f32 = jnp.float32
bf16 = jnp.bfloat16


def _dot(a, b):
    return jnp.dot(a, b, preferred_element_type=f32)


def _dot_tn(a, b):
    return lax.dot_general(a, b, (((0,), (0,)), ((), ())), preferred_element_type=f32)


def _layernorm_t(xt):
    m = jnp.sum(xt, axis=0, keepdims=True) * (1.0 / D)
    d = xt - m
    v = jnp.sum(d * d, axis=0, keepdims=True) * (1.0 / D)
    return d * lax.rsqrt(v + EPS)


def _mish(z):
    sp = jnp.log1p(jnp.exp(-jnp.abs(z))) + jnp.maximum(z, 0.0)
    return z * jnp.tanh(sp)


def _ones_row(pos):
    return 0 if pos == HPG - 1 else MV - 1


def _kernel(x_hbm, wqkv_hbm, wo_hbm, w1_hbm, b1_hbm, w2_hbm, out_ref,
            x_ref, wqkv_ref, wo_ref, w2_ref, k_ref, q_ref, vt_ref, s_ref,
            m_ref, mp_ref, ot_ref, w1_ref, hn_ref, acc_ref, xn_ref, w1t_ref,
            wot_ref, b1_ref, brow_ref, ws_ref, rs_ref, sem):
    blk = pl.program_id(0)

    def cp_x(t):
        return pltpu.make_async_copy(x_hbm.at[:, pl.ds(t * BQ, BQ)], x_ref.at[t], sem.at[t])

    def cp_w1(t):
        cols = pl.ds(t * FQ, FQ)
        return pltpu.make_async_copy(w1_hbm.at[:, cols], w1_ref.at[:, cols], sem.at[NB + t])

    def cp_w2(t, half):
        rows = pl.ds(half * HM + (t % 2) * RQ, RQ)
        cols = pl.ds((t // 2) * FC, FC)
        return pltpu.make_async_copy(w2_hbm.at[rows, cols], w2_ref.at[rows, cols],
                                     sem.at[2 * NB + 2 * t + half])

    cp_wqk = pltpu.make_async_copy(wqkv_hbm.at[:, 0:2 * D], wqkv_ref.at[:, 0:2 * D], sem.at[4 * NB])
    cp_wv = pltpu.make_async_copy(wqkv_hbm.at[:, 2 * D:3 * D], wqkv_ref.at[:, 2 * D:3 * D],
                                  sem.at[4 * NB + 1])
    cp_wo = pltpu.make_async_copy(wo_hbm, wo_ref, sem.at[4 * NB + 2])
    cp_b1 = pltpu.make_async_copy(b1_hbm, b1_ref.at[0:F], sem.at[4 * NB + 3])

    def produce(n, pos, slot, j, mp):
        g = (n % H) // HPG
        keys = slice(j * KC, (j + 1) * KC)
        rows = [q_ref[n], jnp.zeros((128 - 32 - 16 * pos, BQ), bf16)]
        if pos:
            rows.insert(0, jnp.zeros((16 * pos, BQ), bf16))
        s = _dot(k_ref[g, keys, :], jnp.concatenate(rows, axis=0))
        s_ref[slot, keys, :] = s
        sm = jnp.max(s.reshape(KC // 8, 8, BQ), axis=0)
        return sm if mp is None else jnp.maximum(mp, sm)

    def consume(n, slot, j, m, acc):
        keys = slice(j * KC, (j + 1) * KC)
        p = jnp.exp2(s_ref[slot, keys, :] - m).astype(bf16)
        d = _dot(vt_ref[n % H, :, keys], p)
        return d if acc is None else acc + d

    def step(n, u, m, mp):
        par = u % 2
        n1 = jnp.minimum(n + 1, NB * H - 1)
        n2 = jnp.minimum(n + 2, NB * H - 1)
        acc = None
        m_next = None
        for j in range(NCH):
            jp = j + LAG
            if jp < NCH:
                mp = produce(n1, (u + 1) % HPG, 1 - par, jp, mp)
                if jp == NCH - 1:
                    m_next = jnp.max(mp, axis=0, keepdims=True)
                    mp = None
            else:
                mp = produce(n2, (u + 2) % HPG, par, jp - NCH, mp)
            acc = consume(n, par, j, m, acc)
        lrow = _ones_row(u % HPG)
        o = acc * (1.0 / acc[lrow:lrow + 1])
        return m_next, mp, o

    @pl.when(blk == 0)
    def _prologue():
        cp_x(0).start()
        cp_wv.start()
        cp_b1.start()
        cp_wv.wait()
        for t in range(1, NB):
            cp_x(t).start()

        def v_body(t, _):
            tok = pl.ds(pl.multiple_of(t * BQ, BQ), BQ)
            cp_x(t).wait()

            @pl.when(t == 0)
            def _():
                cp_wqk.start()
                for tt in range(NB):
                    cp_w1(tt).start()
                    cp_w2(tt, 0).start()
                    cp_w2(tt, 1).start()
                cp_wo.start()

            xt = x_ref[t].astype(f32)
            xc = xt - jnp.sum(xt, axis=0, keepdims=True) * (1.0 / D)
            rs = lax.rsqrt(jnp.sum(xc * xc, axis=0, keepdims=True) * (1.0 / D) + EPS)
            xn = xc.astype(bf16)
            xn_ref[t] = xn
            rs_ref[t, 0:1, :] = rs
            vt = (_dot_tn(wqkv_ref[:, 2 * D:3 * D], xn) * rs).astype(bf16).astype(f32)
            srow = lax.broadcasted_iota(jnp.int32, (MV, BQ), 0)
            for h in range(H):
                r = 2 * (h % HPG)
                w0 = h * DH - r
                fill = jnp.where(srow == _ones_row(h % HPG), 1.0, 0.0)
                vt_ref[h, :, tok] = jnp.where((srow >= r) & (srow < r + DH), vt[w0:w0 + MV], fill)
            return _

        lax.fori_loop(0, NB, v_body, None)
        cp_b1.wait()
        brow_ref[...] = jnp.concatenate(
            [b1_ref[0:F].astype(f32).reshape(1, F), jnp.zeros((DA - D - 1, F), f32)], axis=0).astype(bf16)
        cp_wqk.wait()
        row = lax.broadcasted_iota(jnp.int32, (32, BQ), 0)

        def qk_body(t, _):
            tok = pl.ds(pl.multiple_of(t * BQ, BQ), BQ)
            cp_w1(t).wait()
            cp_w2(t, 0).wait()
            cp_w2(t, 1).wait()
            xn = xn_ref[t]
            rs = rs_ref[t, 0:1, :]
            QS = 512
            hi_part = _dot_tn(wqkv_ref[:, QS:2 * D], xn) * rs
            for g in range(NG):
                lo = D + g * HPG * DH - QS
                hi = min(lo + 128, 2 * D - QS)
                kg = hi_part[lo:hi]
                if hi - lo < 128:
                    kg = jnp.concatenate([kg, jnp.zeros((128 - (hi - lo), BQ), f32)], axis=0)
                k_ref[g, tok, :] = kg.astype(bf16).T
            q = jnp.concatenate([_dot_tn(wqkv_ref[:, 0:QS], xn) * rs, hi_part[0:D + 32 - QS]], axis=0)
            for h in range(H):
                j = h % HPG
                src = (h // HPG) * HPG * DH + 16 * j
                q_ref[t * H + h] = jnp.where(
                    (row >= 2 * j) & (row < 2 * j + DH), q[src:src + 32] * QSCALE, 0.0).astype(bf16)
            fq = pl.ds(pl.multiple_of(t * FQ, 128), FQ)
            w1t_ref[fq, :] = jnp.concatenate([w1_ref[:, fq], brow_ref[:, fq]], axis=0).T
            c = t // 2
            for rg in range(RQ // 16):
                top = pl.ds(pl.multiple_of((t % 2) * RQ + rg * 16, 16), 16)
                bot = pl.ds(pl.multiple_of(HM + (t % 2) * RQ + rg * 16, 16), 16)
                for lg in range(HF // 384):
                    l1 = pl.ds(pl.multiple_of(c * FC + lg * 384, 128), 384)
                    l2 = pl.ds(pl.multiple_of(c * FC + HF + lg * 384, 128), 384)
                    a11, a12 = w2_ref[top, l1].astype(f32), w2_ref[top, l2].astype(f32)
                    a21, a22 = w2_ref[bot, l1].astype(f32), w2_ref[bot, l2].astype(f32)
                    dst = slice(lg * 384, (lg + 1) * 384)
                    ws_ref[c, 0, top, dst] = (a11 + a22).astype(bf16)
                    ws_ref[c, 1, top, dst] = (a21 + a22).astype(bf16)
                    ws_ref[c, 2, top, dst] = (a11 + a12).astype(bf16)
                    ws_ref[c, 3, top, dst] = (a21 - a11).astype(bf16)
                    ws_ref[c, 4, top, dst] = (a12 - a22).astype(bf16)
            return _

        lax.fori_loop(0, NB, qk_body, None)
        cp_wo.wait()
        wot_ref[...] = wo_ref[...].T
        mp = None
        for j in range(NCH):
            mp = produce(0, 0, 0, j, mp)
        m_ref[0:1, :] = jnp.max(mp, axis=0, keepdims=True)
        mp = None
        for j in range(LAG):
            mp = produce(1, 1, 1, j, mp)
        mp_ref[...] = mp

    def att_body(i, carry):
        m, mp = carry
        og = ot_ref.at[pl.ds(pl.multiple_of(i * UH * DH, 8), UH * DH), :]
        for u in range(UH):
            m, mp, o = step(blk * H + UH * i + u, u, m, mp)
            r = 2 * (u % HPG)
            w0 = u * DH - r
            if r:
                trow = lax.broadcasted_iota(jnp.int32, (8, BQ), 0)
                og[w0:w0 + 8, :] = jnp.where(trow >= r, o[0:8], og[w0:w0 + 8, :])
                og[w0 + 8:w0 + MV, :] = o[8:MV]
            else:
                og[w0:w0 + MV, :] = o
        return m, mp

    m_ref[0:1, :], mp_ref[...] = lax.fori_loop(0, H // UH, att_body, (m_ref[0:1, :], mp_ref[...]))

    ht = x_ref[blk].astype(f32) + _dot(wot_ref[...], ot_ref[...].astype(bf16))
    acc_ref[...] = ht
    hn_ref[0:D, :] = _layernorm_t(ht).astype(bf16)
    hn_ref[D:DA, :] = jnp.concatenate(
        [jnp.ones((1, BQ), f32), jnp.zeros((DA - D - 1, BQ), f32)], axis=0).astype(bf16)

    def ffn_body(c, _):
        fs = pl.ds(pl.multiple_of(c * FC, 128), FC)
        act = _mish(_dot(w1t_ref[fs, :], hn_ref[...]))
        b11, b12 = act[0:HF, 0:HT], act[0:HF, HT:]
        b21, b22 = act[HF:, 0:HT], act[HF:, HT:]
        f1 = pl.ds(pl.multiple_of(c * FC, 128), HF)
        f2 = pl.ds(pl.multiple_of(c * FC + HF, 128), HF)
        mm = lambda a, b: _dot(a, b.astype(bf16))
        m2 = mm(ws_ref[c, 1], b11)
        m6 = mm(ws_ref[c, 3], b11 + b12)
        m5 = mm(ws_ref[c, 2], b22)
        m1 = mm(ws_ref[c, 0], b11 + b22)
        m3 = mm(w2_ref[0:HM, f1], b12 - b22)
        m4 = mm(w2_ref[HM:, f2], b21 - b11)
        m7 = mm(ws_ref[c, 4], b21 + b22)
        top, bot, left, right = slice(0, HM), slice(HM, D), slice(0, HT), slice(HT, BQ)
        for rows, cols, d in ((top, left, (m1 + m4) + (m7 - m5)), (top, right, m3 + m5),
                              (bot, left, m2 + m4), (bot, right, (m1 - m2) + (m3 + m6))):
            v = acc_ref[rows, cols] + d
            acc_ref[rows, cols] = v
            out_ref[rows, cols] = v.astype(bf16)
        return _

    lax.fori_loop(0, F // FC, ffn_body, None)


@jax.jit
def pallas_sequential_preLN__mha_block__dense_activation_mish__prompt_kernel(
    A_x: jax.Array,
    A_wqkv: jax.Array,
    A_wo: jax.Array,
    B_x: jax.Array,
    B_w1: jax.Array,
    B_b1: jax.Array,
    B_w2: jax.Array,
):
    del B_x
    hbm = pl.BlockSpec(memory_space=pltpu.HBM)
    out_t = pl.pallas_call(
        _kernel,
        grid=(NB,),
        in_specs=[hbm] * 6,
        out_specs=pl.BlockSpec((D, BQ), lambda i: (0, i)),
        out_shape=jax.ShapeDtypeStruct((D, S), bf16),
        scratch_shapes=[
            pltpu.VMEM((NB, D, BQ), bf16),
            pltpu.VMEM((D, 3 * D), bf16),
            pltpu.VMEM((D, D), bf16),
            pltpu.VMEM((D, F), bf16),
            pltpu.VMEM((NG, S, 128), bf16),
            pltpu.VMEM((NB * H, 32, BQ), bf16),
            pltpu.VMEM((H, MV, S), f32),
            pltpu.VMEM((2, S, BQ), f32),
            pltpu.VMEM((8, BQ), f32),
            pltpu.VMEM((8, BQ), f32),
            pltpu.VMEM((D, BQ), f32),
            pltpu.VMEM((D, F), bf16),
            pltpu.VMEM((DA, BQ), bf16),
            pltpu.VMEM((D, BQ), f32),
            pltpu.VMEM((NB, D, BQ), bf16),
            pltpu.VMEM((F, DA), bf16),
            pltpu.VMEM((D, D), bf16),
            pltpu.VMEM((F + 1536,), bf16),
            pltpu.VMEM((DA - D, F), bf16),
            pltpu.VMEM((F // FC, 5, HM, HF), bf16),
            pltpu.VMEM((NB, 8, BQ), f32),
            pltpu.SemaphoreType.DMA((4 * NB + 4,)),
        ],
        compiler_params=pltpu.CompilerParams(
            dimension_semantics=("arbitrary",),
            vmem_limit_bytes=100 * 1024 * 1024,
        ),
    )(A_x.reshape(S, D).T, A_wqkv, A_wo, B_w1, B_b1, B_w2.T)
    return out_t.T.reshape(1, S, D)
```
